```python
import jax
import jax.numpy as jnp

def _softmax(x, axis=-1):
    return jax.nn.softmax(x, axis=axis)
def _gelu(x):
    return jax.nn.gelu(x, approximate=True)
def _silu(x):
    return jax.nn.silu(x)
def _sigmoid(x):
    return jax.nn.sigmoid(x)
def _layernorm(x, axis=-1, eps=1e-5):
    m = jnp.mean(x, axis=axis, keepdims=True)
    v = jnp.var(x, axis=axis, keepdims=True)
    return (x - m) / jnp.sqrt(v + eps)
def _scatter_add(tgt, idx, src, axis=0):
    return tgt.at[idx].add(src)
def _segment_sum(src, seg, n):
    return jax.ops.segment_sum(src, seg, n)
class _Rng:
    def __init__(self, key):
        self._k = key
    def _next(self):
        self._k, sub = jax.random.split(self._k)
        return sub
    def normal(self, shape):
        return jax.random.normal(self._next(), shape, dtype=jnp.bfloat16)
    def randint(self, lo, hi, shape):
        return jax.random.randint(self._next(), shape, lo, hi, dtype=jnp.int32)
    def uniform(self, shape, lo=0.0, hi=1.0):
        return jax.random.uniform(self._next(), shape, jnp.bfloat16, lo, hi)
    def permutation(self, n):
        return jax.random.permutation(self._next(), n)


kernel_name = 'gated_mix__compressed_kv_cla__ssm_conv_h3__prompt'

def setup_inputs():
    _rng = _Rng(jax.random.key(int.from_bytes(__import__("os").urandom(4), "little")))
    _w = (lambda a: (lambda t: t.astype(jnp.bfloat16) if jnp.issubdtype(t.dtype, jnp.floating) else t)(jnp.asarray(a)))
    def _A_setup():
        B, H, Sq, Sk, D, M = 1, 32, 2048, 2048, 128, 1024
        Dc = 4 * D
        return {
            "x": _w((lambda *s: _rng.normal(s) * 0.05)(B, Sq, M)),
            "c_kv": _w((lambda *s: _rng.normal(s) * 0.05)(B, Sk, Dc)),
            "w_q": _w((lambda *s: _rng.normal(s) * 0.05)(M, H, D) * (M ** -0.5)),
            "w_uk": _w((lambda *s: _rng.normal(s) * 0.05)(Dc, H, D) * (Dc ** -0.5)),
            "w_uv": _w((lambda *s: _rng.normal(s) * 0.05)(Dc, H, D) * (Dc ** -0.5)),
            "w_o": _w((lambda *s: _rng.normal(s) * 0.05)(H, D, M) * ((H * D) ** -0.5)),
        }
    _A_in = _A_setup()

    def _B_setup():
        B, S, D = 1, 2048, 1024
        ks = 4
        return {
            "q": _w((lambda *s: _rng.normal(s) * 0.05)(B, S, D)),
            "k": _w((lambda *s: _rng.normal(s) * 0.05)(B, S, D)),
            "v": _w((lambda *s: _rng.normal(s) * 0.05)(B, S, D)),
            "shift_k": _w((lambda *s: _rng.normal(s) * 0.05)(D, ks) * 0.5),
            "ssm_k": _w((lambda *s: _rng.normal(s) * 0.05)(D, S) * (1.0 / S ** 0.5)),
            "ssm_D": _w((lambda *s: _rng.normal(s) * 0.05)(D)),
        }
    _B_in = _B_setup()

    return {
        "A_x": _A_in["x"],
        "A_c_kv": _A_in["c_kv"],
        "A_w_q": _A_in["w_q"],
        "A_w_uk": _A_in["w_uk"],
        "A_w_uv": _A_in["w_uv"],
        "A_w_o": _A_in["w_o"],
        "B_q": _B_in["q"],
        "B_k": _B_in["k"],
        "B_v": _B_in["v"],
        "B_shift_k": _B_in["shift_k"],
        "B_ssm_k": _B_in["ssm_k"],
        "B_ssm_D": _B_in["ssm_D"],
        "gate_w": _w((lambda *s: _rng.normal(s) * 0.05)(1024)),
    }

def reference(A_x, A_c_kv, A_w_q, A_w_uk, A_w_uv, A_w_o, B_q, B_k, B_v, B_shift_k, B_ssm_k, B_ssm_D, gate_w):
    def _A_ref(x, c_kv, w_q, w_uk, w_uv, w_o):
        B, Sq, M = x.shape[0], x.shape[1], x.shape[2]
        Sk = c_kv.shape[1]
        H, D = w_q.shape[1], w_q.shape[2]
        q = jnp.einsum("bqm,mhd->bhqd", x, w_q)
        k = jnp.einsum("bkc,chd->bhkd", c_kv, w_uk)
        v = jnp.einsum("bkc,chd->bhkd", c_kv, w_uv)
        scores = jnp.einsum("bhqd,bhkd->bhqk", q, k) * (D ** -0.5)
        off = Sk - Sq
        qi = jnp.arange(Sq)[:, None]
        kj = jnp.arange(Sk)[None, :]
        cmask = kj <= (qi + off)
        scores = jnp.where(cmask[None, None], scores, -1e9)
        p = _softmax(scores, axis=-1)
        ctx = jnp.einsum("bhqk,bhkd->bhqd", p, v)
        return jnp.einsum("bhqd,hdm->bqm", ctx, w_o)

    def _B_ref(q, k, v, shift_k, ssm_k, ssm_D):
        B, S, D = q.shape
        ks = shift_k.shape[-1]
        k_pad = jnp.pad(k, ((0, 0), (ks - 1, 0), (0, 0)))
        k_shift = jnp.zeros_like(k)
        for t in range(ks):
            k_shift = k_shift + k_pad[:, t:t + S, :] * shift_k[:, ks - 1 - t][None, None, :]
        kv = k_shift * v
        L = 2 * S
        kv_pad = jnp.pad(kv, ((0, 0), (0, S), (0, 0)))
        kf_pad = jnp.pad(ssm_k, ((0, 0), (0, S)))
        kv_f = (lambda x, axes=(-2,-1): jnp.fft.rfft2(x.astype(jnp.float32), axes=axes))(kv_pad[:, None, :, :], axes=(1, 2))
        kf_f = (lambda x, axes=(-2,-1): jnp.fft.rfft2(x.astype(jnp.float32), axes=axes))(kf_pad[:, None, :], axes=(1, 2))
        kf_f = (lambda x, *d: x.transpose(*d))(kf_f, 1, 2, 0)
        y_f = kv_f * kf_f[None, :, :, :]
        y = (lambda x, s, axes=(-2,-1): jnp.fft.irfft2(x, s=s, axes=axes).astype(jnp.bfloat16))(y_f, (1, L), axes=(1, 2))[:, 0, :S, :]
        y = y + kv * ssm_D[None, None, :]
        return q * y

    x = A_x
    g = _sigmoid((x * gate_w).sum(-1, keepdims=True))
    a = _A_ref(x, A_c_kv, A_w_q, A_w_uk, A_w_uv, A_w_o)
    b = _B_ref(x, B_k, B_v, B_shift_k, B_ssm_k, B_ssm_D)
    return g * a + (1 - g) * b
```

```python
import numpy as np
import jax
import jax.numpy as jnp
from jax import lax
import jax.experimental.pallas as pl
import jax.experimental.pallas.tpu as pltpu

S = 2048
BQ = 256
HPS = 4


def _consts():
    N = S
    k1 = np.arange(32)
    n1 = np.arange(32)
    n2 = np.arange(64)
    k2 = np.arange(64)
    A = np.exp(-2j * np.pi * np.outer(k1 - 0.25, n1) / 32)
    fa = np.zeros((4, 32, 2, 4, 32))
    for j in range(4):
        fa[j, :, 0, j, :] = A.real
        fa[j, :, 1, j, :] = A.imag
    fa = fa.reshape(256, 128)
    fb = np.zeros((32, 2, 64, 64, 2))
    ib = np.zeros((32, 64, 2, 2, 64))
    for a in range(32):
        G = np.exp(-2j * np.pi * ((a - 0.25) * n2[None, :] / N + np.outer(k2, n2) / 64))
        fb[a, 0, :, :, 0] = G.real
        fb[a, 0, :, :, 1] = -G.imag
        fb[a, 1, :, :, 0] = G.imag
        fb[a, 1, :, :, 1] = G.real
        Gi = np.conj(G).T / 64.0
        ib[a, :, 0, 0, :] = Gi.real
        ib[a, :, 0, 1, :] = -Gi.imag
        ib[a, :, 1, 0, :] = Gi.imag
        ib[a, :, 1, 1, :] = Gi.real
    Ai = np.conj(A).T / 32.0
    ia = np.zeros((2, 32, 2, 32, 2))
    for j in range(2):
        ia[j, :, j, :, 0] = Ai.real
        ia[j, :, j, :, 1] = -Ai.imag
    bf = jnp.bfloat16
    return (fa.astype(bf), fb.reshape(32, 128, 128).astype(bf),
            ib.reshape(32, 128, 128).astype(bf), ia.reshape(64, 128).astype(bf))


def _mm(a, b):
    return jnp.dot(a, b, preferred_element_type=jnp.float32)


def _body(x_ref, c_ref, wq_ref, wk_ref, wv_ref, wo_ref, bk_ref, bv_ref, sh_ref, h_ref, d_ref, g_ref,
          fa_ref, fb_ref, ib_ref, ia_ref, o_ref,
          ctx_ref, y_ref, kp_ref, u_ref, t1_ref, t2_ref, q_ref, k_ref, v_ref):
    step = pl.program_id(0)
    f32, bf = jnp.float32, jnp.bfloat16

    kp_ref[0:8, :] = jnp.zeros((8, 128), f32)
    kp_ref[8:, :] = bk_ref[...].astype(f32)
    sh = sh_ref[...].astype(f32)
    ks = kp_ref[8:, :] * sh[0:1]
    for j in range(1, 4):
        ks = ks + kp_ref[8 - j:8 - j + S, :] * sh[j:j + 1]
    kv = ks * bv_ref[...].astype(f32)
    u_ref[...] = kv
    col = pl.ds(pl.multiple_of(step * 128, 128), 128)
    y_ref[:, col] = kv * d_ref[...].astype(f32)

    def stage_a(t_ref):
        for m in range(16):
            xs = jnp.concatenate(
                [u_ref[pl.ds(4 * m + j, 32, stride=64), :] for j in range(4)], axis=0)
            r = pltpu.bitcast(_mm(fa_ref[...], xs.astype(bf)).astype(bf), jnp.uint32)
            for j in range(4):
                t_ref[pl.ds(4 * m + j, 32, stride=64), :] = r[32 * j:32 * j + 32]

    stage_a(t1_ref)
    u_ref[...] = h_ref[...].astype(f32).T
    stage_a(t2_ref)
    outs = []
    for a in range(32):
        U = _mm(fb_ref[a], pltpu.bitcast(t1_ref[64 * a:64 * a + 64, :], bf))
        H = _mm(fb_ref[a], pltpu.bitcast(t2_ref[64 * a:64 * a + 64, :], bf))
        ur, ui, hr, hi = U[:64], U[64:], H[:64], H[64:]
        P = jnp.concatenate([ur * hr - ui * hi, ur * hi + ui * hr], axis=0).astype(bf)
        kp = pltpu.bitcast(_mm(ib_ref[a], P).astype(bf), jnp.uint32)
        outs.append(kp)
    for a in range(32):
        t1_ref[pl.ds(a, 64, stride=32), :] = outs[a]
    for m in range(32):
        r = _mm(ia_ref[...], pltpu.bitcast(t1_ref[64 * m:64 * m + 64, :], bf))
        for j in range(2):
            u_ref[pl.ds(2 * m + j, 32, stride=64), :] = r[32 * j:32 * j + 32]
    y_ref[:, col] = y_ref[:, col] + u_ref[...]

    row = lax.broadcasted_iota(jnp.int32, (BQ, BQ), 0)
    cl = lax.broadcasted_iota(jnp.int32, (BQ, BQ), 1)

    def head(hh, _):
        hs = pl.ds(pl.multiple_of(hh * 128, 128), 128)
        q_ref[...] = (_mm(x_ref[...], wq_ref[:, hs]) * (128 ** -0.5)).astype(bf)
        k_ref[...] = _mm(c_ref[...], wk_ref[:, hs]).astype(bf)
        v_ref[...] = _mm(c_ref[...], wv_ref[:, hs]).astype(bf)
        oc = pl.ds(pl.multiple_of((step * HPS + hh) * 128, 128), 128)
        for i in range(S // BQ):
            L = (i + 1) * BQ
            s = lax.dot_general(q_ref[i * BQ:L, :], k_ref[0:L, :], (((1,), (1,)), ((), ())),
                                preferred_element_type=f32)
            d = jnp.where(cl <= row, s[:, L - BQ:], -1e9)
            s = d if i == 0 else jnp.concatenate([s[:, :L - BQ], d], axis=1)
            p = jnp.exp(s - jnp.max(s, axis=1, keepdims=True))
            l = jnp.sum(p, axis=1, keepdims=True)
            o = _mm(p.astype(bf), v_ref[0:L, :])
            ctx_ref[i * BQ:L, oc] = (o / l).astype(bf)
        return 0

    lax.fori_loop(0, HPS, head, 0)

    @pl.when(step == pl.num_programs(0) - 1)
    def _():
        def blk(i, _):
            rs = pl.ds(pl.multiple_of(i * 512, 512), 512)
            xf = x_ref[rs, :].astype(f32)
            g = jax.nn.sigmoid(jnp.sum(xf * g_ref[...].astype(f32), axis=1, keepdims=True))
            a = _mm(ctx_ref[rs, :], wo_ref[...])
            o_ref[rs, :] = (g * a + (1 - g) * (xf * y_ref[rs, :])).astype(o_ref.dtype)
            return 0
        lax.fori_loop(0, S // 512, blk, 0)


@jax.jit
def pallas_gated_mix__compressed_kv_cla__ssm_conv_h3__prompt_kernel(
    A_x, A_c_kv, A_w_q, A_w_uk, A_w_uv, A_w_o, B_q, B_k, B_v, B_shift_k, B_ssm_k, B_ssm_D, gate_w,
):
    fa, fb, ib, ia = _consts()
    full = lambda *s: pl.BlockSpec(s, lambda i: (0,) * len(s), pipeline_mode=pl.Buffered(1))
    colb = lambda r, c: pl.BlockSpec((r, c), lambda i: (0, i))
    W = HPS * 128
    out = pl.pallas_call(
        _body,
        grid=(32 // HPS,),
        in_specs=[full(S, 1024), full(S, 512), colb(1024, W), colb(512, W), colb(512, W),
                  full(4096, 1024), colb(S, 128), colb(S, 128), colb(4, 128),
                  pl.BlockSpec((128, S), lambda i: (i, 0)), colb(1, 128), full(1, 1024),
                  full(256, 128), full(32, 128, 128), full(32, 128, 128), full(64, 128)],
        out_specs=pl.BlockSpec((S, 1024), lambda i: (0, 0)),
        out_shape=jax.ShapeDtypeStruct((S, 1024), jnp.bfloat16),
        scratch_shapes=[pltpu.VMEM((S, 4096), jnp.bfloat16), pltpu.VMEM((S, 1024), jnp.float32),
                        pltpu.VMEM((S + 8, 128), jnp.float32), pltpu.VMEM((S, 128), jnp.float32),
                        pltpu.VMEM((S, 128), jnp.uint32), pltpu.VMEM((S, 128), jnp.uint32),
                        pltpu.VMEM((S, 128), jnp.bfloat16), pltpu.VMEM((S, 128), jnp.bfloat16),
                        pltpu.VMEM((S, 128), jnp.bfloat16)],
        compiler_params=pltpu.CompilerParams(dimension_semantics=("arbitrary",),
                                             vmem_limit_bytes=120 * 1024 * 1024),
    )(A_x[0], A_c_kv[0], A_w_q.reshape(1024, 4096), A_w_uk.reshape(512, 4096),
      A_w_uv.reshape(512, 4096), A_w_o.reshape(4096, 1024), B_k[0], B_v[0], B_shift_k.T,
      B_ssm_k, B_ssm_D.reshape(1, 1024), gate_w.reshape(1, 1024), fa, fb, ib, ia)
    return out[None]
```

```python
import numpy as np
import jax
import jax.numpy as jnp
from jax import lax
import jax.experimental.pallas as pl
import jax.experimental.pallas.tpu as pltpu

S = 2048
BQ = 256
HPS = 4


def _consts():
    N = S
    k1 = np.arange(32)
    n1 = np.arange(32)
    n2 = np.arange(64)
    k2 = np.arange(64)
    A = np.exp(-2j * np.pi * np.outer(k1 - 0.25, n1) / 32)
    fa = np.zeros((4, 32, 2, 4, 32))
    for j in range(4):
        fa[j, :, 0, j, :] = A.real
        fa[j, :, 1, j, :] = A.imag
    fa = fa.reshape(256, 128)
    fb = np.zeros((32, 2, 64, 64, 2))
    ib = np.zeros((32, 64, 2, 2, 64))
    for a in range(32):
        G = np.exp(-2j * np.pi * ((a - 0.25) * n2[None, :] / N + np.outer(k2, n2) / 64))
        fb[a, 0, :, :, 0] = G.real
        fb[a, 0, :, :, 1] = -G.imag
        fb[a, 1, :, :, 0] = G.imag
        fb[a, 1, :, :, 1] = G.real
        Gi = np.conj(G).T / 64.0
        ib[a, :, 0, 0, :] = Gi.real
        ib[a, :, 0, 1, :] = -Gi.imag
        ib[a, :, 1, 0, :] = Gi.imag
        ib[a, :, 1, 1, :] = Gi.real
    Ai = np.conj(A).T / 32.0
    ia = np.zeros((2, 32, 2, 32, 2))
    for j in range(2):
        ia[j, :, j, :, 0] = Ai.real
        ia[j, :, j, :, 1] = -Ai.imag
    bf = jnp.bfloat16
    return (fa.astype(bf), fb.reshape(32, 128, 128).astype(bf),
            ib.reshape(32, 128, 128).astype(bf), ia.reshape(64, 128).astype(bf))


def _mm(a, b):
    return jnp.dot(a, b, preferred_element_type=jnp.float32)


def _body(x_ref, c_ref, wq_ref, wk_ref, wv_ref, wo_ref, bk_ref, bv_ref, sh_ref, h_ref, d_ref, g_ref,
          fa_ref, fb_ref, ib_ref, ia_ref, o_ref,
          ctx_ref, y_ref, kp_ref, u_ref, t1_ref, t2_ref, q_ref, k_ref, v_ref, wqs, wks, wvs):
    step = pl.program_id(0)
    f32, bf = jnp.float32, jnp.bfloat16

    kp_ref[0:8, :] = jnp.zeros((8, 128), f32)
    kp_ref[8:, :] = bk_ref[...].astype(f32)
    sh = sh_ref[...].astype(f32)
    ks = kp_ref[8:, :] * sh[0:1]
    for j in range(1, 4):
        ks = ks + kp_ref[8 - j:8 - j + S, :] * sh[j:j + 1]
    kv = ks * bv_ref[...].astype(f32)
    u_ref[...] = kv
    col = pl.ds(pl.multiple_of(step * 128, 128), 128)
    y_ref[:, col] = kv * d_ref[...].astype(f32)

    def stage_a(t_ref):
        for m in range(16):
            xs = jnp.concatenate(
                [u_ref[pl.ds(4 * m + j, 32, stride=64), :] for j in range(4)], axis=0)
            r = pltpu.bitcast(_mm(fa_ref[...], xs.astype(bf)).astype(bf), jnp.uint32)
            for j in range(4):
                t_ref[pl.ds(4 * m + j, 32, stride=64), :] = r[32 * j:32 * j + 32]

    stage_a(t1_ref)
    u_ref[...] = h_ref[...].astype(f32).T
    stage_a(t2_ref)
    outs = []
    for a in range(32):
        U = _mm(fb_ref[a], pltpu.bitcast(t1_ref[64 * a:64 * a + 64, :], bf))
        H = _mm(fb_ref[a], pltpu.bitcast(t2_ref[64 * a:64 * a + 64, :], bf))
        ur, ui, hr, hi = U[:64], U[64:], H[:64], H[64:]
        P = jnp.concatenate([ur * hr - ui * hi, ur * hi + ui * hr], axis=0).astype(bf)
        kp = pltpu.bitcast(_mm(ib_ref[a], P).astype(bf), jnp.uint32)
        outs.append(kp)
    for a in range(32):
        t1_ref[pl.ds(a, 64, stride=32), :] = outs[a]
    for m in range(32):
        r = _mm(ia_ref[...], pltpu.bitcast(t1_ref[64 * m:64 * m + 64, :], bf))
        for j in range(2):
            u_ref[pl.ds(2 * m + j, 32, stride=64), :] = r[32 * j:32 * j + 32]
    y_ref[:, col] = y_ref[:, col] + u_ref[...]

    row = lax.broadcasted_iota(jnp.int32, (BQ, BQ), 0)
    cl = lax.broadcasted_iota(jnp.int32, (BQ, BQ), 1)

    @pl.when(step % 2 == 0)
    def _():
        for src, dst in ((wq_ref, wqs), (wk_ref, wks), (wv_ref, wvs)):
            for r in range(0, src.shape[0], 128):
                dst[r * 8:r * 8 + 1024, :] = src[r:r + 128].astype(f32).reshape(1024, 128)

    def head(hh, _):
        h8 = (step % 2) * HPS + hh
        q_ref[...] = (_mm(x_ref[...], wqs[pl.ds(h8, 1024, stride=8), :].astype(bf)) * (128 ** -0.5)).astype(bf)
        k_ref[...] = _mm(c_ref[...], wks[pl.ds(h8, 512, stride=8), :].astype(bf)).astype(bf)
        v_ref[...] = _mm(c_ref[...], wvs[pl.ds(h8, 512, stride=8), :].astype(bf)).astype(bf)
        oc = pl.ds(pl.multiple_of((step * HPS + hh) * 128, 128), 128)
        for i in range(S // BQ):
            L = (i + 1) * BQ
            s = lax.dot_general(q_ref[i * BQ:L, :], k_ref[0:L, :], (((1,), (1,)), ((), ())),
                                preferred_element_type=f32)
            d = jnp.where(cl <= row, s[:, L - BQ:], -1e9)
            s = d if i == 0 else jnp.concatenate([s[:, :L - BQ], d], axis=1)
            p = jnp.exp(s - jnp.max(s, axis=1, keepdims=True))
            l = jnp.sum(p, axis=1, keepdims=True)
            o = _mm(p.astype(bf), v_ref[0:L, :])
            ctx_ref[i * BQ:L, oc] = (o / l).astype(bf)
        return 0

    lax.fori_loop(0, HPS, head, 0)

    @pl.when(step == pl.num_programs(0) - 1)
    def _():
        def blk(i, _):
            rs = pl.ds(pl.multiple_of(i * 512, 512), 512)
            xf = x_ref[rs, :].astype(f32)
            g = jax.nn.sigmoid(jnp.sum(xf * g_ref[...].astype(f32), axis=1, keepdims=True))
            a = _mm(ctx_ref[rs, :], wo_ref[...])
            o_ref[rs, :] = (g * a + (1 - g) * (xf * y_ref[rs, :])).astype(o_ref.dtype)
            return 0
        lax.fori_loop(0, S // 512, blk, 0)


@jax.jit
def pallas_gated_mix__compressed_kv_cla__ssm_conv_h3__prompt_kernel(
    A_x, A_c_kv, A_w_q, A_w_uk, A_w_uv, A_w_o, B_q, B_k, B_v, B_shift_k, B_ssm_k, B_ssm_D, gate_w,
):
    fa, fb, ib, ia = _consts()
    full = lambda *s: pl.BlockSpec(s, lambda i: (0,) * len(s), pipeline_mode=pl.Buffered(1))
    colb = lambda r, c: pl.BlockSpec((r, c), lambda i: (0, i))
    w3 = lambda r: pl.BlockSpec((r, 8, 128), lambda i: (0, i // 2, 0))
    out = pl.pallas_call(
        _body,
        grid=(32 // HPS,),
        in_specs=[full(S, 1024), full(S, 512), w3(1024), w3(512), w3(512),
                  full(4096, 1024), colb(S, 128), colb(S, 128), colb(4, 128),
                  pl.BlockSpec((128, S), lambda i: (i, 0)), colb(1, 128), full(1, 1024),
                  full(256, 128), full(32, 128, 128), full(32, 128, 128), full(64, 128)],
        out_specs=pl.BlockSpec((S, 1024), lambda i: (0, 0)),
        out_shape=jax.ShapeDtypeStruct((S, 1024), jnp.bfloat16),
        scratch_shapes=[pltpu.VMEM((S, 4096), jnp.bfloat16), pltpu.VMEM((S, 1024), jnp.float32),
                        pltpu.VMEM((S + 8, 128), jnp.float32), pltpu.VMEM((S, 128), jnp.float32),
                        pltpu.VMEM((S, 128), jnp.uint32), pltpu.VMEM((S, 128), jnp.uint32),
                        pltpu.VMEM((S, 128), jnp.bfloat16), pltpu.VMEM((S, 128), jnp.bfloat16),
                        pltpu.VMEM((S, 128), jnp.bfloat16), pltpu.VMEM((8192, 128), jnp.float32),
                        pltpu.VMEM((4096, 128), jnp.float32), pltpu.VMEM((4096, 128), jnp.float32)],
        compiler_params=pltpu.CompilerParams(dimension_semantics=("arbitrary",),
                                             vmem_limit_bytes=120 * 1024 * 1024),
    )(A_x[0], A_c_kv[0], A_w_q, A_w_uk,
      A_w_uv, A_w_o.reshape(4096, 1024), B_k[0], B_v[0], B_shift_k.T,
      B_ssm_k, B_ssm_D.reshape(1, 1024), gate_w.reshape(1, 1024), fa, fb, ib, ia)
    return out[None]
```

```python
import numpy as np
import jax
import jax.numpy as jnp
from jax import lax
import jax.experimental.pallas as pl
import jax.experimental.pallas.tpu as pltpu

S = 2048
BQ = 256
HPS = 4


def _consts():
    N = S
    k1 = np.arange(32)
    n1 = np.arange(32)
    n2 = np.arange(64)
    k2 = np.arange(64)
    A = np.exp(-2j * np.pi * np.outer(k1 - 0.25, n1) / 32)
    fa = np.zeros((4, 32, 2, 4, 32))
    for j in range(4):
        fa[j, :, 0, j, :] = A.real
        fa[j, :, 1, j, :] = A.imag
    fa = fa.reshape(256, 128)
    fb = np.zeros((32, 2, 64, 64, 2))
    ib = np.zeros((32, 64, 2, 2, 64))
    for a in range(32):
        G = np.exp(-2j * np.pi * ((a - 0.25) * n2[None, :] / N + np.outer(k2, n2) / 64))
        fb[a, 0, :, :, 0] = G.real
        fb[a, 0, :, :, 1] = -G.imag
        fb[a, 1, :, :, 0] = G.imag
        fb[a, 1, :, :, 1] = G.real
        Gi = np.conj(G).T / 64.0
        ib[a, :, 0, 0, :] = Gi.real
        ib[a, :, 0, 1, :] = -Gi.imag
        ib[a, :, 1, 0, :] = Gi.imag
        ib[a, :, 1, 1, :] = Gi.real
    Ai = np.conj(A).T / 32.0
    ia = np.zeros((2, 32, 2, 32, 2))
    for j in range(2):
        ia[j, :, j, :, 0] = Ai.real
        ia[j, :, j, :, 1] = -Ai.imag
    bf = jnp.bfloat16
    return (fa.astype(bf), fb.reshape(32, 128, 128).astype(bf),
            ib.reshape(32, 128, 128).astype(bf), ia.reshape(64, 128).astype(bf))


def _mm(a, b):
    return jnp.dot(a, b, preferred_element_type=jnp.float32)


def _body(x_ref, c_ref, wq_ref, wk_ref, wv_ref, wo_hbm, bk_ref, bv_ref, sh_ref, h_ref, d_ref, g_ref,
          fa_ref, fb_ref, ib_ref, ia_ref, o_ref,
          ctx_ref, y_ref, kp_ref, u_ref, t1_ref, t2_ref, q_ref, k_ref, v_ref, wqs, wks, wvs, wo_ref, sem):
    step = pl.program_id(0)
    wo_cp = pltpu.make_async_copy(wo_hbm, wo_ref, sem)
    pl.when(step == 1)(wo_cp.start)
    f32, bf = jnp.float32, jnp.bfloat16

    kp_ref[0:8, :] = jnp.zeros((8, 128), f32)
    kp_ref[8:, :] = bk_ref[...].astype(f32)
    sh = sh_ref[...].astype(f32)
    ks = kp_ref[8:, :] * sh[0:1]
    for j in range(1, 4):
        ks = ks + kp_ref[8 - j:8 - j + S, :] * sh[j:j + 1]
    kv = ks * bv_ref[...].astype(f32)
    u_ref[...] = kv
    col = pl.ds(pl.multiple_of(step * 128, 128), 128)
    y_ref[:, col] = kv * d_ref[...].astype(f32)

    def stage_a(t_ref):
        for m in range(16):
            xs = jnp.concatenate(
                [u_ref[pl.ds(4 * m + j, 32, stride=64), :] for j in range(4)], axis=0)
            r = pltpu.bitcast(_mm(fa_ref[...], xs.astype(bf)).astype(bf), jnp.uint32)
            for j in range(4):
                t_ref[pl.ds(4 * m + j, 32, stride=64), :] = r[32 * j:32 * j + 32]

    stage_a(t1_ref)
    u_ref[...] = h_ref[...].astype(f32).T
    stage_a(t2_ref)
    outs = []
    for a in range(32):
        U = _mm(fb_ref[a], pltpu.bitcast(t1_ref[64 * a:64 * a + 64, :], bf))
        H = _mm(fb_ref[a], pltpu.bitcast(t2_ref[64 * a:64 * a + 64, :], bf))
        ur, ui, hr, hi = U[:64], U[64:], H[:64], H[64:]
        P = jnp.concatenate([ur * hr - ui * hi, ur * hi + ui * hr], axis=0).astype(bf)
        kp = pltpu.bitcast(_mm(ib_ref[a], P).astype(bf), jnp.uint32)
        outs.append(kp)
    for a in range(32):
        t1_ref[pl.ds(a, 64, stride=32), :] = outs[a]
    for m in range(32):
        r = _mm(ia_ref[...], pltpu.bitcast(t1_ref[64 * m:64 * m + 64, :], bf))
        for j in range(2):
            u_ref[pl.ds(2 * m + j, 32, stride=64), :] = r[32 * j:32 * j + 32]
    y_ref[:, col] = y_ref[:, col] + u_ref[...]

    row = lax.broadcasted_iota(jnp.int32, (BQ, BQ), 0)
    cl = lax.broadcasted_iota(jnp.int32, (BQ, BQ), 1)

    @pl.when(step % 2 == 0)
    def _():
        for src, dst in ((wq_ref, wqs), (wk_ref, wks), (wv_ref, wvs)):
            for r in range(0, src.shape[0], 128):
                dst[r * 8:r * 8 + 1024, :] = src[r:r + 128].astype(f32).reshape(1024, 128)

    def head(hh, _):
        h8 = (step % 2) * HPS + hh
        q_ref[...] = (_mm(x_ref[...], wqs[pl.ds(h8, 1024, stride=8), :].astype(bf)) * (128 ** -0.5 * 1.4426950408889634)).astype(bf)
        k_ref[...] = _mm(c_ref[...], wks[pl.ds(h8, 512, stride=8), :].astype(bf)).astype(bf)
        v_ref[...] = _mm(c_ref[...], wvs[pl.ds(h8, 512, stride=8), :].astype(bf)).astype(bf)
        oc = pl.ds(pl.multiple_of((step * HPS + hh) * 128, 128), 128)
        for i in range(S // BQ):
            L = (i + 1) * BQ
            s = lax.dot_general(q_ref[i * BQ:L, :], k_ref[0:L, :], (((1,), (1,)), ((), ())),
                                preferred_element_type=f32)
            d = jnp.where(cl <= row, s[:, L - BQ:], -1e9)
            s = d if i == 0 else jnp.concatenate([s[:, :L - BQ], d], axis=1)
            p = jnp.exp2(s - jnp.max(s, axis=1, keepdims=True))
            l = jnp.sum(p, axis=1, keepdims=True)
            o = _mm(p.astype(bf), v_ref[0:L, :])
            ctx_ref[i * BQ:L, oc] = (o * (1.0 / l)).astype(bf)
        return 0

    lax.fori_loop(0, HPS, head, 0)

    @pl.when(step == pl.num_programs(0) - 1)
    def _():
        wo_cp.wait()

        def blk(i, _):
            rs = pl.ds(pl.multiple_of(i * 512, 512), 512)
            xf = x_ref[rs, :].astype(f32)
            g = jax.nn.sigmoid(jnp.sum(xf * g_ref[...].astype(f32), axis=1, keepdims=True))
            a = _mm(ctx_ref[rs, :], wo_ref[...])
            o_ref[rs, :] = (g * a + (1 - g) * (xf * y_ref[rs, :])).astype(o_ref.dtype)
            return 0
        lax.fori_loop(0, S // 512, blk, 0)


@jax.jit
def pallas_gated_mix__compressed_kv_cla__ssm_conv_h3__prompt_kernel(
    A_x, A_c_kv, A_w_q, A_w_uk, A_w_uv, A_w_o, B_q, B_k, B_v, B_shift_k, B_ssm_k, B_ssm_D, gate_w,
):
    fa, fb, ib, ia = _consts()
    full = lambda *s: pl.BlockSpec(s, lambda i: (0,) * len(s), pipeline_mode=pl.Buffered(1))
    colb = lambda r, c: pl.BlockSpec((r, c), lambda i: (0, i))
    w3 = lambda r: pl.BlockSpec((r, 8, 128), lambda i: (0, i // 2, 0))
    out = pl.pallas_call(
        _body,
        grid=(32 // HPS,),
        in_specs=[full(S, 1024), full(S, 512), w3(1024), w3(512), w3(512),
                  pl.BlockSpec(memory_space=pl.ANY), colb(S, 128), colb(S, 128), colb(4, 128),
                  pl.BlockSpec((128, S), lambda i: (i, 0)), colb(1, 128), full(1, 1024),
                  full(256, 128), full(32, 128, 128), full(32, 128, 128), full(64, 128)],
        out_specs=pl.BlockSpec((S, 1024), lambda i: (0, 0)),
        out_shape=jax.ShapeDtypeStruct((S, 1024), jnp.bfloat16),
        scratch_shapes=[pltpu.VMEM((S, 4096), jnp.bfloat16), pltpu.VMEM((S, 1024), jnp.float32),
                        pltpu.VMEM((S + 8, 128), jnp.float32), pltpu.VMEM((S, 128), jnp.float32),
                        pltpu.VMEM((S, 128), jnp.uint32), pltpu.VMEM((S, 128), jnp.uint32),
                        pltpu.VMEM((S, 128), jnp.bfloat16), pltpu.VMEM((S, 128), jnp.bfloat16),
                        pltpu.VMEM((S, 128), jnp.bfloat16), pltpu.VMEM((8192, 128), jnp.float32),
                        pltpu.VMEM((4096, 128), jnp.float32), pltpu.VMEM((4096, 128), jnp.float32),
 pltpu.VMEM((4096, 1024), jnp.bfloat16), pltpu.SemaphoreType.DMA(())],
        compiler_params=pltpu.CompilerParams(dimension_semantics=("arbitrary",),
                                             vmem_limit_bytes=120 * 1024 * 1024),
    )(A_x[0], A_c_kv[0], A_w_q, A_w_uk,
      A_w_uv, A_w_o.reshape(4096, 1024), B_k[0], B_v[0], B_shift_k.T,
      B_ssm_k, B_ssm_D.reshape(1, 1024), gate_w.reshape(1, 1024), fa, fb, ib, ia)
    return out[None]
```

```python
import numpy as np
import jax
import jax.numpy as jnp
from jax import lax
import jax.experimental.pallas as pl
import jax.experimental.pallas.tpu as pltpu

S = 2048
BQ = 256
HPS = 4


def _consts():
    N = S
    k1 = np.arange(32)
    n1 = np.arange(32)
    n2 = np.arange(64)
    k2 = np.arange(64)
    A = np.exp(-2j * np.pi * np.outer(k1 - 0.25, n1) / 32)
    fa = np.zeros((4, 32, 2, 4, 32))
    for j in range(4):
        fa[j, :, 0, j, :] = A.real
        fa[j, :, 1, j, :] = A.imag
    fa = fa.reshape(256, 128)
    fb = np.zeros((32, 2, 64, 64, 2))
    ib = np.zeros((32, 64, 2, 2, 64))
    for a in range(32):
        G = np.exp(-2j * np.pi * ((a - 0.25) * n2[None, :] / N + np.outer(k2, n2) / 64))
        fb[a, 0, :, :, 0] = G.real
        fb[a, 0, :, :, 1] = -G.imag
        fb[a, 1, :, :, 0] = G.imag
        fb[a, 1, :, :, 1] = G.real
        Gi = np.conj(G).T / 64.0
        ib[a, :, 0, 0, :] = Gi.real
        ib[a, :, 0, 1, :] = -Gi.imag
        ib[a, :, 1, 0, :] = Gi.imag
        ib[a, :, 1, 1, :] = Gi.real
    Ai = np.conj(A).T / 32.0
    ia = np.zeros((2, 32, 2, 32, 2))
    for j in range(2):
        ia[j, :, j, :, 0] = Ai.real
        ia[j, :, j, :, 1] = -Ai.imag
    bf = jnp.bfloat16
    return (fa.astype(bf), fb.reshape(32, 128, 128).astype(bf),
            ib.reshape(32, 128, 128).astype(bf), ia.reshape(64, 128).astype(bf))


def _mm(a, b):
    return jnp.dot(a, b, preferred_element_type=jnp.float32)


def _body(x_ref, c_ref, wq_ref, wk_ref, wv_ref, wo_hbm, bk_ref, bv_ref, sh_ref, h_ref, d_ref, g_ref,
          fa_ref, fb_ref, ib_ref, ia_ref, o_ref,
          ctx_ref, y_ref, kp_ref, u_ref, t1_ref, t2_ref, q_ref, k_ref, v_ref, wqs, wks, wvs, wo_ref, sem, t3_ref):
    step = pl.program_id(0)
    wo_cp = pltpu.make_async_copy(wo_hbm, wo_ref, sem)
    pl.when(step == 1)(wo_cp.start)
    f32, bf = jnp.float32, jnp.bfloat16

    kp_ref[0:8, :] = jnp.zeros((8, 128), f32)
    kp_ref[8:, :] = bk_ref[...].astype(f32)
    sh = sh_ref[...].astype(f32)
    ks = kp_ref[8:, :] * sh[0:1]
    for j in range(1, 4):
        ks = ks + kp_ref[8 - j:8 - j + S, :] * sh[j:j + 1]
    kv = ks * bv_ref[...].astype(f32)
    u_ref[...] = kv
    col = pl.ds(pl.multiple_of(step * 128, 128), 128)
    y_ref[:, col] = kv * d_ref[...].astype(f32)

    def stage_a(t_ref):
        for m in range(16):
            xs = jnp.concatenate(
                [u_ref[pl.ds(4 * m + j, 32, stride=64), :] for j in range(4)], axis=0)
            r = pltpu.bitcast(_mm(fa_ref[...], xs.astype(bf)).astype(bf), jnp.uint32)
            for j in range(4):
                t_ref[pl.ds(4 * m + j, 32, stride=64), :] = r[32 * j:32 * j + 32]

    stage_a(t1_ref)
    u_ref[...] = h_ref[...].astype(f32).T
    stage_a(t2_ref)
    row = lax.broadcasted_iota(jnp.int32, (BQ, BQ), 0)
    cl = lax.broadcasted_iota(jnp.int32, (BQ, BQ), 1)

    @pl.when(step % 2 == 0)
    def _():
        for src, dst in ((wq_ref, wqs), (wk_ref, wks), (wv_ref, wvs)):
            for r in range(0, src.shape[0], 128):
                dst[r * 8:r * 8 + 1024, :] = src[r:r + 128].astype(f32).reshape(1024, 128)

    def head(hh, _):
        for aa in range(8):
            a = hh * 8 + aa
            rs = pl.ds(pl.multiple_of(a * 64, 64), 64)
            U = _mm(fb_ref[a], pltpu.bitcast(t1_ref[rs, :], bf))
            H = _mm(fb_ref[a], pltpu.bitcast(t2_ref[rs, :], bf))
            ur, ui, hr, hi = U[:64], U[64:], H[:64], H[64:]
            P = jnp.concatenate([ur * hr - ui * hi, ur * hi + ui * hr], axis=0).astype(bf)
            t3_ref[pl.ds(a, 64, stride=32), :] = pltpu.bitcast(_mm(ib_ref[a], P).astype(bf), jnp.uint32)
        h8 = (step % 2) * HPS + hh
        q_ref[...] = (_mm(x_ref[...], wqs[pl.ds(h8, 1024, stride=8), :].astype(bf)) * (128 ** -0.5 * 1.4426950408889634)).astype(bf)
        k_ref[...] = _mm(c_ref[...], wks[pl.ds(h8, 512, stride=8), :].astype(bf)).astype(bf)
        v_ref[...] = _mm(c_ref[...], wvs[pl.ds(h8, 512, stride=8), :].astype(bf)).astype(bf)
        oc = pl.ds(pl.multiple_of((step * HPS + hh) * 128, 128), 128)
        for i in range(S // BQ):
            L = (i + 1) * BQ
            s = lax.dot_general(q_ref[i * BQ:L, :], k_ref[0:L, :], (((1,), (1,)), ((), ())),
                                preferred_element_type=f32)
            d = jnp.where(cl <= row, s[:, L - BQ:], -1e9)
            s = d if i == 0 else jnp.concatenate([s[:, :L - BQ], d], axis=1)
            p = jnp.exp2(s - jnp.max(s, axis=1, keepdims=True))
            l = jnp.sum(p, axis=1, keepdims=True)
            o = _mm(p.astype(bf), v_ref[0:L, :])
            ctx_ref[i * BQ:L, oc] = (o * (1.0 / l)).astype(bf)
        return 0

    lax.fori_loop(0, HPS, head, 0)
    for m in range(32):
        r = _mm(ia_ref[...], pltpu.bitcast(t3_ref[64 * m:64 * m + 64, :], bf))
        for j in range(2):
            u_ref[pl.ds(2 * m + j, 32, stride=64), :] = r[32 * j:32 * j + 32]
    y_ref[:, col] = y_ref[:, col] + u_ref[...]


    @pl.when(step == pl.num_programs(0) - 1)
    def _():
        wo_cp.wait()

        def blk(i, _):
            rs = pl.ds(pl.multiple_of(i * 512, 512), 512)
            xf = x_ref[rs, :].astype(f32)
            g = jax.nn.sigmoid(jnp.sum(xf * g_ref[...].astype(f32), axis=1, keepdims=True))
            a = _mm(ctx_ref[rs, :], wo_ref[...])
            o_ref[rs, :] = (g * a + (1 - g) * (xf * y_ref[rs, :])).astype(o_ref.dtype)
            return 0
        lax.fori_loop(0, S // 512, blk, 0)


@jax.jit
def pallas_gated_mix__compressed_kv_cla__ssm_conv_h3__prompt_kernel(
    A_x, A_c_kv, A_w_q, A_w_uk, A_w_uv, A_w_o, B_q, B_k, B_v, B_shift_k, B_ssm_k, B_ssm_D, gate_w,
):
    fa, fb, ib, ia = _consts()
    full = lambda *s: pl.BlockSpec(s, lambda i: (0,) * len(s), pipeline_mode=pl.Buffered(1))
    colb = lambda r, c: pl.BlockSpec((r, c), lambda i: (0, i))
    w3 = lambda r: pl.BlockSpec((r, 8, 128), lambda i: (0, i // 2, 0))
    out = pl.pallas_call(
        _body,
        grid=(32 // HPS,),
        in_specs=[full(S, 1024), full(S, 512), w3(1024), w3(512), w3(512),
                  pl.BlockSpec(memory_space=pl.ANY), colb(S, 128), colb(S, 128), colb(4, 128),
                  pl.BlockSpec((128, S), lambda i: (i, 0)), colb(1, 128), full(1, 1024),
                  full(256, 128), full(32, 128, 128), full(32, 128, 128), full(64, 128)],
        out_specs=pl.BlockSpec((S, 1024), lambda i: (0, 0)),
        out_shape=jax.ShapeDtypeStruct((S, 1024), jnp.bfloat16),
        scratch_shapes=[pltpu.VMEM((S, 4096), jnp.bfloat16), pltpu.VMEM((S, 1024), jnp.float32),
                        pltpu.VMEM((S + 8, 128), jnp.float32), pltpu.VMEM((S, 128), jnp.float32),
                        pltpu.VMEM((S, 128), jnp.uint32), pltpu.VMEM((S, 128), jnp.uint32),
                        pltpu.VMEM((S, 128), jnp.bfloat16), pltpu.VMEM((S, 128), jnp.bfloat16),
                        pltpu.VMEM((S, 128), jnp.bfloat16), pltpu.VMEM((8192, 128), jnp.float32),
                        pltpu.VMEM((4096, 128), jnp.float32), pltpu.VMEM((4096, 128), jnp.float32),
 pltpu.VMEM((4096, 1024), jnp.bfloat16), pltpu.SemaphoreType.DMA(()), pltpu.VMEM((S, 128), jnp.uint32)],
        compiler_params=pltpu.CompilerParams(dimension_semantics=("arbitrary",),
                                             vmem_limit_bytes=120 * 1024 * 1024),
    )(A_x[0], A_c_kv[0], A_w_q, A_w_uk,
      A_w_uv, A_w_o.reshape(4096, 1024), B_k[0], B_v[0], B_shift_k.T,
      B_ssm_k, B_ssm_D.reshape(1, 1024), gate_w.reshape(1, 1024), fa, fb, ib, ia)
    return out[None]
```

```python
import numpy as np
import jax
import jax.numpy as jnp
from jax import lax
import jax.experimental.pallas as pl
import jax.experimental.pallas.tpu as pltpu

S = 2048
BQ = 256
HPS = 4


def _consts():
    N = S
    k1 = np.arange(32)
    n1 = np.arange(32)
    n2 = np.arange(64)
    k2 = np.arange(64)
    A = np.exp(-2j * np.pi * np.outer(k1 - 0.25, n1) / 32)
    fa = np.zeros((4, 32, 2, 4, 32))
    for j in range(4):
        fa[j, :, 0, j, :] = A.real
        fa[j, :, 1, j, :] = A.imag
    fa = fa.reshape(256, 128)
    fb = np.zeros((32, 2, 64, 64, 2))
    ib = np.zeros((32, 64, 2, 2, 64))
    for a in range(32):
        G = np.exp(-2j * np.pi * ((a - 0.25) * n2[None, :] / N + np.outer(k2, n2) / 64))
        fb[a, 0, :, :, 0] = G.real
        fb[a, 0, :, :, 1] = -G.imag
        fb[a, 1, :, :, 0] = G.imag
        fb[a, 1, :, :, 1] = G.real
        Gi = np.conj(G).T / 64.0
        ib[a, :, 0, 0, :] = Gi.real
        ib[a, :, 0, 1, :] = -Gi.imag
        ib[a, :, 1, 0, :] = Gi.imag
        ib[a, :, 1, 1, :] = Gi.real
    Ai = np.conj(A).T / 32.0
    ia = np.zeros((2, 32, 2, 32, 2))
    for j in range(2):
        ia[j, :, j, :, 0] = Ai.real
        ia[j, :, j, :, 1] = -Ai.imag
    bf = jnp.bfloat16
    return (fa.astype(bf), fb.reshape(32, 128, 128).astype(bf),
            ib.reshape(32, 128, 128).astype(bf), ia.reshape(64, 128).astype(bf))


def _mm(a, b):
    return jnp.dot(a, b, preferred_element_type=jnp.float32)


def _body(x_ref, c_ref, wq_ref, wk_ref, wv_ref, wo_hbm, bk_ref, bv_ref, sh_ref, h_ref, d_ref, g_ref,
          fa_ref, fb_ref, ib_ref, ia_ref, o_ref,
          ctx_ref, y_ref, kp_ref, u_ref, t1_ref, t2_ref, q_ref, k_ref, v_ref, wqs, wks, wvs, wo_ref, sem, t3_ref):
    step = pl.program_id(0)
    wo_cp = pltpu.make_async_copy(wo_hbm, wo_ref, sem)
    pl.when(step == 1)(wo_cp.start)
    f32, bf = jnp.float32, jnp.bfloat16

    kp_ref[0:8, :] = jnp.zeros((8, 128), f32)
    kp_ref[8:, :] = bk_ref[...].astype(f32)
    sh = sh_ref[...].astype(f32)
    ks = kp_ref[8:, :] * sh[0:1]
    for j in range(1, 4):
        ks = ks + kp_ref[8 - j:8 - j + S, :] * sh[j:j + 1]
    kv = ks * bv_ref[...].astype(f32)
    def put(val):
        for b in range(32):
            u_ref[65 * b:65 * b + 64, :] = val[64 * b:64 * b + 64]
    put(kv)
    col = pl.ds(pl.multiple_of(step * 128, 128), 128)
    y_ref[:, col] = kv * d_ref[...].astype(f32)

    def stage_a(t_ref):
        for m in range(16):
            xs = jnp.concatenate(
                [u_ref[pl.ds(4 * m + j, 32, stride=65), :] for j in range(4)], axis=0)
            r = pltpu.bitcast(_mm(fa_ref[...], xs.astype(bf)).astype(bf), jnp.uint32)
            for j in range(4):
                t_ref[pl.ds(4 * m + j, 32, stride=65), :] = r[32 * j:32 * j + 32]

    stage_a(t1_ref)
    put(h_ref[...].astype(f32).T)
    stage_a(t2_ref)
    row = lax.broadcasted_iota(jnp.int32, (BQ, BQ), 0)
    cl = lax.broadcasted_iota(jnp.int32, (BQ, BQ), 1)

    @pl.when(step % 2 == 0)
    def _():
        for src, dst in ((wq_ref, wqs), (wk_ref, wks), (wv_ref, wvs)):
            for r in range(0, src.shape[0], 128):
                dst[r * 8:r * 8 + 1024, :] = src[r:r + 128].astype(f32).reshape(1024, 128)

    def head(hh, _):
        for aa in range(8):
            a = hh * 8 + aa
            rs = pl.ds(a * 65, 64)
            U = _mm(fb_ref[a], pltpu.bitcast(t1_ref[rs, :], bf))
            H = _mm(fb_ref[a], pltpu.bitcast(t2_ref[rs, :], bf))
            ur, ui, hr, hi = U[:64], U[64:], H[:64], H[64:]
            P = jnp.concatenate([ur * hr - ui * hi, ur * hi + ui * hr], axis=0).astype(bf)
            t3_ref[pl.ds(a, 64, stride=33), :] = pltpu.bitcast(_mm(ib_ref[a], P).astype(bf), jnp.uint32)
        h8 = (step % 2) * HPS + hh
        q_ref[...] = (_mm(x_ref[...], wqs[pl.ds(h8, 1024, stride=8), :].astype(bf)) * (128 ** -0.5 * 1.4426950408889634)).astype(bf)
        k_ref[...] = _mm(c_ref[...], wks[pl.ds(h8, 512, stride=8), :].astype(bf)).astype(bf)
        v_ref[...] = _mm(c_ref[...], wvs[pl.ds(h8, 512, stride=8), :].astype(bf)).astype(bf)
        oc = pl.ds(pl.multiple_of((step * HPS + hh) * 128, 128), 128)
        for i in range(S // BQ):
            L = (i + 1) * BQ
            s = lax.dot_general(q_ref[i * BQ:L, :], k_ref[0:L, :], (((1,), (1,)), ((), ())),
                                preferred_element_type=f32)
            d = jnp.where(cl <= row, s[:, L - BQ:], -1e9)
            s = d if i == 0 else jnp.concatenate([s[:, :L - BQ], d], axis=1)
            p = jnp.exp2(s - jnp.max(s, axis=1, keepdims=True))
            l = jnp.sum(p, axis=1, keepdims=True)
            o = _mm(p.astype(bf), v_ref[0:L, :])
            ctx_ref[i * BQ:L, oc] = (o * (1.0 / l)).astype(bf)
        return 0

    lax.fori_loop(0, HPS, head, 0)
    for m in range(32):
        r = _mm(ia_ref[...], pltpu.bitcast(jnp.concatenate([t3_ref[66 * m:66 * m + 32, :], t3_ref[66 * m + 33:66 * m + 65, :]], axis=0), bf))
        for j in range(2):
            u_ref[pl.ds(2 * m + j, 32, stride=65), :] = r[32 * j:32 * j + 32]
    y_ref[:, col] = y_ref[:, col] + jnp.concatenate([u_ref[65 * b:65 * b + 64, :] for b in range(32)], axis=0)


    @pl.when(step == pl.num_programs(0) - 1)
    def _():
        wo_cp.wait()

        def blk(i, _):
            rs = pl.ds(pl.multiple_of(i * 512, 512), 512)
            xf = x_ref[rs, :].astype(f32)
            g = jax.nn.sigmoid(jnp.sum(xf * g_ref[...].astype(f32), axis=1, keepdims=True))
            a = _mm(ctx_ref[rs, :], wo_ref[...])
            o_ref[rs, :] = (g * a + (1 - g) * (xf * y_ref[rs, :])).astype(o_ref.dtype)
            return 0
        lax.fori_loop(0, S // 512, blk, 0)


@jax.jit
def pallas_gated_mix__compressed_kv_cla__ssm_conv_h3__prompt_kernel(
    A_x, A_c_kv, A_w_q, A_w_uk, A_w_uv, A_w_o, B_q, B_k, B_v, B_shift_k, B_ssm_k, B_ssm_D, gate_w,
):
    fa, fb, ib, ia = _consts()
    full = lambda *s: pl.BlockSpec(s, lambda i: (0,) * len(s), pipeline_mode=pl.Buffered(1))
    colb = lambda r, c: pl.BlockSpec((r, c), lambda i: (0, i))
    w3 = lambda r: pl.BlockSpec((r, 8, 128), lambda i: (0, i // 2, 0))
    out = pl.pallas_call(
        _body,
        grid=(32 // HPS,),
        in_specs=[full(S, 1024), full(S, 512), w3(1024), w3(512), w3(512),
                  pl.BlockSpec(memory_space=pl.ANY), colb(S, 128), colb(S, 128), colb(4, 128),
                  pl.BlockSpec((128, S), lambda i: (i, 0)), colb(1, 128), full(1, 1024),
                  full(256, 128), full(32, 128, 128), full(32, 128, 128), full(64, 128)],
        out_specs=pl.BlockSpec((S, 1024), lambda i: (0, 0)),
        out_shape=jax.ShapeDtypeStruct((S, 1024), jnp.bfloat16),
        scratch_shapes=[pltpu.VMEM((S, 4096), jnp.bfloat16), pltpu.VMEM((S, 1024), jnp.float32),
                        pltpu.VMEM((S + 8, 128), jnp.float32), pltpu.VMEM((S + 32, 128), jnp.float32),
                        pltpu.VMEM((S + 64, 128), jnp.uint32), pltpu.VMEM((S + 64, 128), jnp.uint32),
                        pltpu.VMEM((S, 128), jnp.bfloat16), pltpu.VMEM((S, 128), jnp.bfloat16),
                        pltpu.VMEM((S, 128), jnp.bfloat16), pltpu.VMEM((8192, 128), jnp.float32),
                        pltpu.VMEM((4096, 128), jnp.float32), pltpu.VMEM((4096, 128), jnp.float32),
 pltpu.VMEM((4096, 1024), jnp.bfloat16), pltpu.SemaphoreType.DMA(()), pltpu.VMEM((S + 64, 128), jnp.uint32)],
        compiler_params=pltpu.CompilerParams(dimension_semantics=("arbitrary",),
                                             vmem_limit_bytes=120 * 1024 * 1024),
    )(A_x[0], A_c_kv[0], A_w_q, A_w_uk,
      A_w_uv, A_w_o.reshape(4096, 1024), B_k[0], B_v[0], B_shift_k.T,
      B_ssm_k, B_ssm_D.reshape(1, 1024), gate_w.reshape(1, 1024), fa, fb, ib, ia)
    return out[None]
```
